```python
import os as _os
_os.environ.setdefault("JAX_PLATFORMS", "cpu")
import jax
import jax.numpy as jnp

def _softmax(x, axis=-1):
    return jax.nn.softmax(x, axis=axis)
def _gelu(x):
    return jax.nn.gelu(x, approximate=True)
def _silu(x):
    return jax.nn.silu(x)
def _sigmoid(x):
    return jax.nn.sigmoid(x)
def _layernorm(x, axis=-1, eps=1e-5):
    m = jnp.mean(x, axis=axis, keepdims=True)
    v = jnp.var(x, axis=axis, keepdims=True)
    return (x - m) / jnp.sqrt(v + eps)
def _scatter_add(tgt, idx, src, axis=0):
    return tgt.at[idx].add(src)
def _segment_sum(src, seg, n):
    return jax.ops.segment_sum(src, seg, n)
class _Rng:
    def __init__(self, key):
        self._k = key
    def _next(self):
        self._k, sub = jax.random.split(self._k)
        return sub
    def normal(self, shape):
        return jax.random.normal(self._next(), shape, dtype=jnp.bfloat16)
    def randint(self, lo, hi, shape):
        return jax.random.randint(self._next(), shape, lo, hi, dtype=jnp.int32)
    def uniform(self, shape, lo=0.0, hi=1.0):
        return jax.random.uniform(self._next(), shape, jnp.bfloat16, lo, hi)
    def permutation(self, n):
        return jax.random.permutation(self._next(), n)


kernel_name = 'standalone__mha_softmax__near_ridge'

def setup_inputs():
    _rng = _Rng(jax.random.key(int.from_bytes(__import__("os").urandom(4), "little")))
    _w = (lambda a: (lambda t: t.astype(jnp.bfloat16) if jnp.issubdtype(t.dtype, jnp.floating) else t)(jnp.asarray(a)))
    B, H, Sq, Sk, D = 8, 32, 384, 512, 128
    return {
        "q": _w((lambda *s: _rng.normal(s) * 0.4)(B, H, Sq, D)),
        "k": _w((lambda *s: _rng.normal(s) * 0.4)(B, H, Sk, D)),
        "v": _w((lambda *s: _rng.normal(s) * 0.05)(B, H, Sk, D)),
    }

def reference(q, k, v):
    scale = q.shape[-1] ** -0.5
    scores = jnp.einsum("bhqd,bhkd->bhqk", q, k) * scale
    p = _softmax(scores, axis=-1)
    return jnp.einsum("bhqk,bhkd->bhqd", p, v)
```

```python
import jax
import jax.numpy as jnp
from jax import lax
import jax.experimental.pallas as pl
import jax.experimental.pallas.tpu as pltpu

_LOG2E = 1.4426950408889634

_HEADS_PER_STEP = 4
_READ_GROUP = 5
_READS_AHEAD = 3
_WRITE_GROUP = 15
_WRITES_BEHIND = 3
_READ_SPLIT = 4
_NUM_SEMS = 16


def _attend(q, k, v):
    scale = q.shape[-1] ** -0.5 * _LOG2E
    s = lax.dot_general(
        q, k, (((1,), (1,)), ((), ())), preferred_element_type=jnp.float32
    )
    m = jnp.max(s, axis=-1, keepdims=True)
    p = jnp.exp2((s - m) * scale)
    l = jnp.sum(p, axis=-1, keepdims=True)
    o = jnp.dot(p.astype(v.dtype), v, preferred_element_type=jnp.float32)
    r = pl.reciprocal(l, approx=True)
    r = r * (2.0 - l * r)
    return (o * r).astype(q.dtype)


@jax.jit
def pallas_standalone__mha_softmax__near_ridge_kernel(
    q: jax.Array,
    k: jax.Array,
    v: jax.Array,
):
    B, H, Sq, D = q.shape
    Sk = k.shape[2]
    nh = B * H
    rows = Sq + 2 * Sk

    G, RG, RA = _HEADS_PER_STEP, _READ_GROUP, _READS_AHEAD
    WG, WB, NS = _WRITE_GROUP, _WRITES_BEHIND, _NUM_SEMS

    n_read_groups = nh // RG
    first = nh - (n_read_groups - 1) * RG
    steps1 = n_read_groups - RA
    heads1 = steps1 * G
    steps2 = (nh - heads1) // G
    assert (nh - heads1) % G == 0 and first >= G
    assert steps2 * WG <= min(nh, heads1 + (steps2 - 1) * G) and steps2 > max(RA, WB)

    def kernel(q_hbm, k_hbm, v_hbm, o_hbm, qkv, out, read_sems, write_sems):
        operands = ((q_hbm, Sq, 0), (k_hbm, Sk, Sq), (v_hbm, Sk, Sq + Sk))

        def group_start(j):
            return first + (j - 1) * RG

        def start_reads(h0, n, slot):
            issued = 0
            for i in range(n):
                h = h0 + i
                for c in range(_READ_SPLIT):
                    for src, seq, base in operands:
                        chunk = seq // _READ_SPLIT
                        pltpu.make_async_copy(
                            src.at[pl.ds(h * seq + c * chunk, chunk)],
                            qkv.at[h, pl.ds(base + c * chunk, chunk)],
                            read_sems.at[slot],
                        ).start(priority=issued % 2)
                        issued += 1

        def wait_reads(h0, n, slot):
            filled = qkv.at[pl.ds(h0, n)]
            pltpu.make_async_copy(filled, filled, read_sems.at[slot]).wait()

        def start_writes(h0, n, slot):
            for i in range(n):
                pltpu.make_async_copy(
                    out.at[h0 + i], o_hbm.at[h0 + i], write_sems.at[slot]
                ).start(priority=i % 2)

        def wait_writes(h0, n, slot):
            pltpu.make_async_copy(
                out.at[pl.ds(h0, n)], o_hbm.at[pl.ds(h0, n)], write_sems.at[slot]
            ).wait()

        def compute(h):
            out[h] = _attend(
                qkv[h, 0:Sq, :], qkv[h, Sq:Sq + Sk, :], qkv[h, Sq + Sk:rows, :]
            )

        start_reads(0, first, 0)
        for j in range(1, RA):
            start_reads(group_start(j), RG, j)
        wait_reads(0, first, 0)

        def read_phase(t, carry):
            @pl.when(t > 0)
            def _():
                wait_reads(group_start(t), RG, t & (NS - 1))

            for g in range(G):
                compute(t * G + g)
            start_reads(group_start(t + RA), RG, (t + RA) & (NS - 1))
            return carry

        lax.fori_loop(0, steps1, read_phase, None)

        def write_phase(t, carry):
            @pl.when(t < RA)
            def _():
                wait_reads(group_start(steps1 + t), RG, (steps1 + t) & (NS - 1))

            @pl.when(t >= WB)
            def _():
                wait_writes((t - WB) * WG, WG, (t - WB) & (NS - 1))

            start_writes(t * WG, WG, t & (NS - 1))
            for g in range(G):
                compute(heads1 + t * G + g)
            return carry

        lax.fori_loop(0, steps2, write_phase, None)

        rest = nh - steps2 * WG
        if rest:
            start_writes(steps2 * WG, rest, steps2 % NS)
        for t in range(steps2 - WB, steps2):
            wait_writes(t * WG, WG, t % NS)
        if rest:
            wait_writes(steps2 * WG, rest, steps2 % NS)

    out = pl.pallas_call(
        kernel,
        in_specs=[pl.BlockSpec(memory_space=pl.ANY)] * 3,
        out_specs=pl.BlockSpec(memory_space=pl.ANY),
        out_shape=jax.ShapeDtypeStruct((nh, Sq, D), q.dtype),
        scratch_shapes=[
            pltpu.VMEM((nh, rows, D), q.dtype),
            pltpu.VMEM((nh, Sq, D), q.dtype),
            pltpu.SemaphoreType.DMA((NS,)),
            pltpu.SemaphoreType.DMA((NS,)),
        ],
        compiler_params=pltpu.CompilerParams(
            vmem_limit_bytes=127 * 2**20,
            disable_bounds_checks=True,
        ),
    )(q.reshape(nh * Sq, D), k.reshape(nh * Sk, D), v.reshape(nh * Sk, D))
    return out.reshape(B, H, Sq, D)
```

```python
import jax
import jax.numpy as jnp
from jax import lax
import jax.experimental.pallas as pl
import jax.experimental.pallas.tpu as pltpu

_LOG2E = 1.4426950408889634

_STREAMS = 8
_STEP_HEADS = 4
_PARTS = 4
_STEP_BLOCKS = 5
_FIRST_BLOCKS = 11
_READS_AFTER = (24, 36, 48, 60)
_WRITE_ROWS = 128
_INPUT_SLOTS = 16


def _attend(q, k, v):
    scale = q.shape[-1] ** -0.5 * _LOG2E
    s = lax.dot_general(
        q, k, (((1,), (1,)), ((), ())), preferred_element_type=jnp.float32
    )
    m = jnp.max(s, axis=-1, keepdims=True)
    p = jnp.exp2((s - m) * scale)
    l = jnp.sum(p, axis=-1, keepdims=True)
    o = jnp.dot(p.astype(v.dtype), v, preferred_element_type=jnp.float32)
    r = pl.reciprocal(l, approx=True)
    r = r * (2.0 - l * r)
    return (o * r).astype(q.dtype)


def _log2(n):
    assert n & (n - 1) == 0
    return n.bit_length() - 1


@jax.jit
def pallas_standalone__mha_softmax__near_ridge_kernel(
    q: jax.Array,
    k: jax.Array,
    v: jax.Array,
):
    B, H, Sq, D = q.shape
    Sk = k.shape[2]

    S, G, P, E = _STREAMS, _STEP_HEADS, _PARTS, _STEP_BLOCKS
    depth = B * H // S
    steps = B * H // G
    sweep = S // G
    read_steps = (steps * P - _FIRST_BLOCKS) // E
    assert depth * S == B * H and sweep * G == S and Sq % P == 0 and Sk % P == 0
    assert read_steps * E + _FIRST_BLOCKS == steps * P
    assert P <= min(E, _FIRST_BLOCKS) and read_steps + 1 < steps
    assert steps - read_steps < _INPUT_SLOTS

    kq, qq = Sk // P, Sq // P
    k_part, v_part, q_part = (0, kq), (kq, kq), (2 * kq, qq)
    block_dmas = 3 * G

    def kernel(q_hbm, k_hbm, v_hbm, o_hbm, qkv, out, read_sems, write_sem):
        def locate(t):
            return (t & (sweep - 1)) * G, t >> _log2(sweep)

        def slot(t):
            return t & (_INPUT_SLOTS - 1)

        def start_reads(first_block, lo, hi):
            for i in range(lo // block_dmas, pl.cdiv(hi, block_dmas)):
                t, part = (first_block + i) >> _log2(P), (first_block + i) & (P - 1)
                stream, pos = locate(t)
                dmas = [
                    (g, src, row, rows)
                    for g in range(G)
                    for src, (row, rows) in (
                        (k_hbm, k_part), (v_hbm, v_part), (q_hbm, q_part)
                    )
                ]
                for j, (g, src, row, rows) in enumerate(dmas):
                    if lo <= i * block_dmas + j < hi:
                        pltpu.make_async_copy(
                            src.at[stream + g, pos, pl.ds(part * rows, rows)],
                            qkv.at[slot(t), part, g, pl.ds(row, rows)],
                            read_sems.at[slot(t)],
                        ).start(priority=j % 2)

        def wait_reads(t):
            filled = qkv.at[slot(t)]
            pltpu.make_async_copy(filled, filled, read_sems.at[slot(t)]).wait()

        def start_writes(pos):
            for row in range(0, Sq, _WRITE_ROWS):
                rows = pl.ds(row, _WRITE_ROWS)
                pltpu.make_async_copy(
                    out.at[:, pos, rows], o_hbm.at[:, pos, rows], write_sem.at[0]
                ).start()

        def compute(t, g):
            def load(row, rows):
                parts = [qkv[slot(t), p, g, row:row + rows, :] for p in range(P)]
                return jnp.concatenate(parts, axis=0)

            stream, pos = locate(t)
            out[stream + g, pos] = _attend(load(*q_part), load(*k_part), load(*v_part))

        start_reads(0, 0, _FIRST_BLOCKS * block_dmas)

        def read_step(t, carry):
            wait_reads(t)
            issued = 0
            for g in range(G):
                compute(t, g)
                start_reads(_FIRST_BLOCKS + t * E, issued, _READS_AFTER[g])
                issued = _READS_AFTER[g]
            return carry

        lax.fori_loop(0, read_steps, read_step, None)

        def written(t):
            return jnp.where(t > read_steps, t >> _log2(sweep), 0)

        def write_step(t, carry):
            wait_reads(t)
            lax.fori_loop(
                written(t - 1), written(t), lambda pos, _: start_writes(pos), None
            )
            for g in range(G):
                compute(t, g)
            return carry

        lax.fori_loop(read_steps, steps, write_step, None)

        for pos in range((steps - 1) // sweep, depth):
            start_writes(pos)
        pltpu.make_async_copy(out, o_hbm, write_sem.at[0]).wait()

    out = pl.pallas_call(
        kernel,
        in_specs=[pl.BlockSpec(memory_space=pl.ANY)] * 3,
        out_specs=pl.BlockSpec(memory_space=pl.ANY),
        out_shape=jax.ShapeDtypeStruct((S, depth, Sq, D), q.dtype),
        scratch_shapes=[
            pltpu.VMEM((_INPUT_SLOTS, P, G, qq + 2 * kq, D), q.dtype),
            pltpu.VMEM((S, depth, Sq, D), q.dtype),
            pltpu.SemaphoreType.DMA((_INPUT_SLOTS,)),
            pltpu.SemaphoreType.DMA((1,)),
        ],
        compiler_params=pltpu.CompilerParams(
            vmem_limit_bytes=64 * 2**20,
            disable_bounds_checks=True,
            disable_semaphore_checks=True,
        ),
    )(
        q.reshape(S, depth, Sq, D),
        k.reshape(S, depth, Sk, D),
        v.reshape(S, depth, Sk, D),
    )
    return out.reshape(B, H, Sq, D)
```
